```python
import os as _os
_os.environ.setdefault("JAX_PLATFORMS", "cpu")
import jax
import jax.numpy as jnp

def _softmax(x, axis=-1):
    return jax.nn.softmax(x, axis=axis)
def _gelu(x):
    return jax.nn.gelu(x, approximate=True)
def _silu(x):
    return jax.nn.silu(x)
def _sigmoid(x):
    return jax.nn.sigmoid(x)
def _layernorm(x, axis=-1, eps=1e-5):
    m = jnp.mean(x, axis=axis, keepdims=True)
    v = jnp.var(x, axis=axis, keepdims=True)
    return (x - m) / jnp.sqrt(v + eps)
def _scatter_add(tgt, idx, src, axis=0):
    return tgt.at[idx].add(src)
def _segment_sum(src, seg, n):
    return jax.ops.segment_sum(src, seg, n)
class _Rng:
    def __init__(self, key):
        self._k = key
    def _next(self):
        self._k, sub = jax.random.split(self._k)
        return sub
    def normal(self, shape):
        return jax.random.normal(self._next(), shape, dtype=jnp.bfloat16)
    def randint(self, lo, hi, shape):
        return jax.random.randint(self._next(), shape, lo, hi, dtype=jnp.int32)
    def uniform(self, shape, lo=0.0, hi=1.0):
        return jax.random.uniform(self._next(), shape, jnp.bfloat16, lo, hi)
    def permutation(self, n):
        return jax.random.permutation(self._next(), n)


kernel_name = 'gated_mix__linear_attn_block__glu_gated_swiglu__prompt'

def setup_inputs():
    _rng = _Rng(jax.random.key(int.from_bytes(__import__("os").urandom(4), "little")))
    _w = (lambda a: (lambda t: t.astype(jnp.bfloat16) if jnp.issubdtype(t.dtype, jnp.floating) else t)(jnp.asarray(a)))
    def _A_setup():
        B, S, D = 1, 2048, 1024
        return {
            "x": _w((lambda *s: _rng.normal(s) * 0.05)(B, S, D)),
            "wqkv": _w((lambda *s: _rng.normal(s) * 0.8)(D, 3 * D)),
            "wo": _w((lambda *s: _rng.normal(s) * 0.05)(D, D)),
        }
    _A_in = _A_setup()

    def _B_setup():
        B, S, D, F = 1, 2048, 1024, 3584
        return {
            "x": _w((lambda *s: _rng.normal(s) * 0.05)(B, S, D)),
            "w1": _w((lambda *s: _rng.normal(s) * 1.6)(D, F) * (2.0 / D) ** 0.5),
            "w3": _w((lambda *s: _rng.normal(s) * 1.6)(D, F) * (2.0 / D) ** 0.5),
            "w2": _w((lambda *s: _rng.normal(s) * 1.6)(F, D) * (2.0 / F) ** 0.5),
        }
    _B_in = _B_setup()

    return {
        "A_x": _A_in["x"],
        "A_wqkv": _A_in["wqkv"],
        "A_wo": _A_in["wo"],
        "B_x": _B_in["x"],
        "B_w1": _B_in["w1"],
        "B_w3": _B_in["w3"],
        "B_w2": _B_in["w2"],
        "gate_w": _w((lambda *s: _rng.normal(s) * 0.05)(1024) * 16.0),
    }

def reference(A_x, A_wqkv, A_wo, B_x, B_w1, B_w3, B_w2, gate_w):
    def _A_ref(x, wqkv, wo):
        B, S, D = x.shape
        H = 32; Dh = D // H
        qkv = (lambda x, *d: x.transpose(*d))((x @ wqkv).reshape(B, S, 3, H, Dh), 2, 0, 3, 1, 4)
        q, k, v = qkv[0], qkv[1], qkv[2]
        phi = lambda t: jnp.where(t > 0, t + 1, jnp.exp(t)) + 1e-6
        pq, pk = phi(q), phi(k)
        kv = jnp.einsum("bhsd,bhse->bhde", pk, v)
        z = jnp.einsum("bhsd->bhd", pk)
        num = jnp.einsum("bhqd,bhde->bhqe", pq, kv)
        den = jnp.einsum("bhqd,bhd->bhq", pq, z)[..., None] + 1e-6
        o = num / den
        return (lambda x, *d: x.transpose(*d))(o, 0, 2, 1, 3).reshape(B, S, D) @ wo

    def _B_ref(x, w1, w3, w2):
        gate = jnp.einsum("bsd,df->bsf", x, w1)
        up = jnp.einsum("bsd,df->bsf", x, w3)
        h = _silu(gate) * up
        out = jnp.einsum("bsf,fd->bsd", h, w2)
        return out

    x = A_x
    g = _sigmoid((x * gate_w).sum(-1, keepdims=True))
    a = _A_ref(x, A_wqkv, A_wo)
    b = _B_ref(x, B_w1, B_w3, B_w2)
    return g * a + (1 - g) * b
```

```python
import functools

import jax
import jax.numpy as jnp
from jax import lax
import jax.experimental.pallas as pl
import jax.experimental.pallas.tpu as pltpu

HEAD_DIM = 32
LANE = 128


def _phi(t):
    return jnp.where(t > 0, t + 1.0, jnp.exp(t)) + 1e-6


def _kernel(x_hbm, wqkv_hbm, wo_hbm, w1_hbm, w3_hbm, w2_hbm, gw_ref,
            o_ref,
            x_v, wq_v, wkv_v, wo_v, w1_v, w3_v, w2_v,
            kv_acc, z_acc, m_v, zexp_v, sems,
            *, tm, n1, n2, S, D, F, fc):
    i = pl.program_id(0)
    nblk = D // LANE

    def x_copy(t):
        return pltpu.make_async_copy(
            x_hbm.at[pl.ds(t * tm, tm), :], x_v.at[pl.ds(t * tm, tm), :], sems.at[t])

    def wk_copy():
        return pltpu.make_async_copy(
            wqkv_hbm.at[:, pl.ds(D, D)], wkv_v.at[:, pl.ds(0, D)], sems.at[n1])

    def wv_copy():
        return pltpu.make_async_copy(
            wqkv_hbm.at[:, pl.ds(2 * D, D)], wkv_v.at[:, pl.ds(D, D)], sems.at[n1 + 1])

    def late_copies():
        return [
            pltpu.make_async_copy(wqkv_hbm.at[:, pl.ds(0, D)], wq_v, sems.at[n1 + 2]),
            pltpu.make_async_copy(wo_hbm, wo_v, sems.at[n1 + 3]),
            pltpu.make_async_copy(w1_hbm, w1_v, sems.at[n1 + 4]),
            pltpu.make_async_copy(w3_hbm, w3_v, sems.at[n1 + 5]),
            pltpu.make_async_copy(w2_hbm, w2_v, sems.at[n1 + 6]),
        ]

    @pl.when(i == 0)
    def _():
        x_copy(0).start()
        wk_copy().start()
        wv_copy().start()
        for t in range(1, n1):
            x_copy(t).start()
        for c in late_copies():
            c.start()
        kv_acc[...] = jnp.zeros_like(kv_acc)
        z_acc[...] = jnp.zeros_like(z_acc)
        wk_copy().wait()
        wv_copy().wait()

    @pl.when(i < n1)
    def _():
        for t in range(n1):
            @pl.when(i == t)
            def _():
                x_copy(t).wait()
        r0 = pl.multiple_of(i * tm, tm)
        xt = x_v[pl.ds(r0, tm), :]
        k = jnp.dot(xt, wkv_v[:, pl.ds(0, D)], preferred_element_type=jnp.float32)
        pk = _phi(k).astype(jnp.bfloat16)
        v = jnp.dot(xt, wkv_v[:, pl.ds(D, D)],
                    preferred_element_type=jnp.float32).astype(jnp.bfloat16)
        z_acc[...] += jnp.sum(pk.astype(jnp.float32), axis=0, keepdims=True)
        for j in range(nblk):
            kv_acc[j] += lax.dot_general(
                pk[:, j * LANE:(j + 1) * LANE], v[:, j * LANE:(j + 1) * LANE],
                (((0,), (0,)), ((), ())), preferred_element_type=jnp.float32)

    @pl.when(i == n1)
    def _():
        for c in late_copies():
            c.wait()
        rr = lax.broadcasted_iota(jnp.int32, (LANE, LANE), 0) // HEAD_DIM
        cc = lax.broadcasted_iota(jnp.int32, (LANE, LANE), 1) // HEAD_DIM
        diag = rr == cc
        for j in range(nblk):
            kvj = jnp.where(diag, kv_acc[j], 0.0).astype(jnp.bfloat16)
            m_v[pl.ds(j * LANE, LANE), :] = jnp.dot(
                kvj, wo_v[pl.ds(j * LANE, LANE), :],
                preferred_element_type=jnp.float32).astype(jnp.bfloat16)
            zrow = jnp.broadcast_to(z_acc[:, pl.ds(j * LANE, LANE)], (LANE, LANE))
            zexp_v[j] = jnp.where(diag, zrow.T, 0.0).astype(jnp.bfloat16)

    @pl.when(i >= n1)
    def _():
        r0 = pl.multiple_of((i - n1) * tm, tm)
        xt = x_v[pl.ds(r0, tm), :]
        q = jnp.dot(xt, wq_v[...], preferred_element_type=jnp.float32)
        pq = _phi(q).astype(jnp.bfloat16)
        parts = []
        for j in range(nblk):
            pqj = pq[:, j * LANE:(j + 1) * LANE]
            den = jnp.dot(pqj, zexp_v[j], preferred_element_type=jnp.float32) + 1e-6
            parts.append((pqj.astype(jnp.float32) / den).astype(jnp.bfloat16))
        pqn = jnp.concatenate(parts, axis=1)
        a = jnp.dot(pqn, m_v[...], preferred_element_type=jnp.float32)

        def body(c, acc):
            c0 = pl.multiple_of(c * fc, fc)
            gate = jnp.dot(xt, w1_v[:, pl.ds(c0, fc)], preferred_element_type=jnp.float32)
            up = jnp.dot(xt, w3_v[:, pl.ds(c0, fc)], preferred_element_type=jnp.float32)
            h = (gate * jax.nn.sigmoid(gate) * up).astype(jnp.bfloat16)
            return acc + jnp.dot(h, w2_v[pl.ds(c0, fc), :],
                                 preferred_element_type=jnp.float32)

        b = lax.fori_loop(0, F // fc, body, jnp.zeros((tm, D), jnp.float32))
        gw = gw_ref[...].astype(jnp.float32)
        g = jax.nn.sigmoid(jnp.sum(xt.astype(jnp.float32) * gw, axis=-1, keepdims=True))
        o_ref[...] = (g * a + (1.0 - g) * b).astype(o_ref.dtype)


@jax.jit
def pallas_gated_mix__linear_attn_block__glu_gated_swiglu__prompt_kernel(
    A_x: jax.Array,
    A_wqkv: jax.Array,
    A_wo: jax.Array,
    B_x: jax.Array,
    B_w1: jax.Array,
    B_w3: jax.Array,
    B_w2: jax.Array,
    gate_w: jax.Array,
):
    B, S, D = A_x.shape
    F = B_w1.shape[1]
    tm = 512
    fc = 512
    n1 = S // tm
    n2 = S // tm
    x2 = A_x.reshape(S, D)
    gw2 = gate_w.reshape(1, D)
    bf = jnp.bfloat16

    kernel = functools.partial(_kernel, tm=tm, n1=n1, n2=n2, S=S, D=D, F=F, fc=fc)
    any_spec = pl.BlockSpec(memory_space=pl.ANY)
    out = pl.pallas_call(
        kernel,
        grid=(n1 + n2,),
        in_specs=[any_spec] * 6 + [pl.BlockSpec((1, D), lambda i: (0, 0))],
        out_specs=pl.BlockSpec((tm, D), lambda i: (jnp.maximum(i - n1, 0), 0)),
        out_shape=jax.ShapeDtypeStruct((S, D), A_x.dtype),
        scratch_shapes=[
            pltpu.VMEM((S, D), bf),
            pltpu.VMEM((D, D), bf),
            pltpu.VMEM((D, 2 * D), bf),
            pltpu.VMEM((D, D), bf),
            pltpu.VMEM((D, F), bf),
            pltpu.VMEM((D, F), bf),
            pltpu.VMEM((F, D), bf),
            pltpu.VMEM((D // LANE, LANE, LANE), jnp.float32),
            pltpu.VMEM((1, D), jnp.float32),
            pltpu.VMEM((D, D), bf),
            pltpu.VMEM((D // LANE, LANE, LANE), bf),
            pltpu.SemaphoreType.DMA((n1 + 7,)),
        ],
        compiler_params=pltpu.CompilerParams(
            dimension_semantics=("arbitrary",),
            vmem_limit_bytes=100 * 1024 * 1024,
        ),
    )(x2, A_wqkv, A_wo, B_w1, B_w3, B_w2, gw2)
    return out.reshape(B, S, D)
```

```python
import functools

import jax
import jax.numpy as jnp
from jax import lax
import jax.experimental.pallas as pl
import jax.experimental.pallas.tpu as pltpu

HEAD_DIM = 32
LANE = 128


def _phi(t):
    return jnp.where(t > 0, t + 1.0, jnp.exp(t)) + 1e-6


def _kernel(x_hbm, wqkv_hbm, wo_hbm, w1_hbm, w3_hbm, w2_hbm, gw_ref,
            o_ref,
            x_v, wq_v, wk_v, wv_v, wo_v, w1_v, w3_v, w2_v,
            p_acc, z_acc, m_v, gw_v, sems,
            *, t1, nt1, kc, nc1, tm, n2, S, D, F, fc):
    i = pl.program_id(0)
    n1 = nt1 * nc1
    nblk = D // LANE
    bpc = kc // LANE

    def x_copy(t):
        return pltpu.make_async_copy(
            x_hbm.at[pl.ds(t * t1, t1), :], x_v.at[pl.ds(t * t1, t1), :], sems.at[t])

    def wk_copy(c):
        return pltpu.make_async_copy(
            wqkv_hbm.at[:, pl.ds(D + c * kc, kc)], wk_v.at[c], sems.at[nt1 + c])

    sb = nt1 + nc1

    def late_copies():
        return [
            pltpu.make_async_copy(wqkv_hbm.at[:, pl.ds(2 * D, D)], wv_v, sems.at[sb]),
            pltpu.make_async_copy(wo_hbm, wo_v, sems.at[sb + 1]),
            pltpu.make_async_copy(wqkv_hbm.at[:, pl.ds(0, D)], wq_v, sems.at[sb + 2]),
            pltpu.make_async_copy(w1_hbm, w1_v, sems.at[sb + 3]),
            pltpu.make_async_copy(w3_hbm, w3_v, sems.at[sb + 4]),
            pltpu.make_async_copy(w2_hbm, w2_v, sems.at[sb + 5]),
        ]

    @pl.when(i == 0)
    def _():
        x_copy(0).start()
        wk_copy(0).start()
        for t in range(1, nt1):
            x_copy(t).start()
        for c in range(1, nc1):
            wk_copy(c).start()
        for c in late_copies():
            c.start()
        p_acc[...] = jnp.zeros_like(p_acc)
        z_acc[...] = jnp.zeros_like(z_acc)
        gw_v[...] = gw_ref[...].astype(jnp.float32).reshape(1, D)

    @pl.when(i < n1)
    def _():
        c = i // nt1
        t = i % nt1
        for tt in range(nt1):
            @pl.when(i == tt)
            def _():
                x_copy(tt).wait()
        for cc in range(nc1):
            @pl.when(i == cc * nt1)
            def _():
                wk_copy(cc).wait()
        r0 = pl.multiple_of(t * t1, t1)
        xt = x_v[pl.ds(r0, t1), :]
        k = jnp.dot(xt, wk_v[c], preferred_element_type=jnp.float32)
        pk = _phi(k).astype(jnp.bfloat16)
        z_acc[c] += jnp.sum(pk.astype(jnp.float32), axis=0, keepdims=True)
        p_acc[c] += lax.dot_general(
            pk, xt, (((0,), (0,)), ((), ())), preferred_element_type=jnp.float32)

    @pl.when(i == n1)
    def _():
        for c in late_copies():
            c.wait()
        rr = lax.broadcasted_iota(jnp.int32, (LANE, LANE), 0) // HEAD_DIM
        cc = lax.broadcasted_iota(jnp.int32, (LANE, LANE), 1) // HEAD_DIM
        diag = rr == cc
        for j in range(nblk):
            pj = p_acc[j // bpc, pl.ds((j % bpc) * LANE, LANE), :].astype(jnp.bfloat16)
            kvj = jnp.dot(pj, wv_v[:, pl.ds(j * LANE, LANE)],
                          preferred_element_type=jnp.float32)
            kvj = jnp.where(diag, kvj, 0.0).astype(jnp.bfloat16)
            m_v[pl.ds(j * LANE, LANE), :] = jnp.dot(
                kvj, wo_v[pl.ds(j * LANE, LANE), :],
                preferred_element_type=jnp.float32).astype(jnp.bfloat16)

    @pl.when(i >= n1)
    def _():
        r0 = pl.multiple_of((i - n1) * tm, tm)
        xt = x_v[pl.ds(r0, tm), :]
        q = jnp.dot(xt, wq_v[...], preferred_element_type=jnp.float32)
        gate = jnp.dot(xt, w1_v[:, pl.ds(0, fc)], preferred_element_type=jnp.float32)
        pq = _phi(q).astype(jnp.bfloat16)
        parts = []
        lane = lax.broadcasted_iota(jnp.int32, (tm, LANE), 1)
        for j in range(nblk):
            pqj = pq[:, j * LANE:(j + 1) * LANE].astype(jnp.float32)
            y = pqj * z_acc[j // bpc, :, pl.ds((j % bpc) * LANE, LANE)]
            s = 1
            while s < HEAD_DIM:
                fwd = pltpu.roll(y, s, 1)
                bwd = pltpu.roll(y, LANE - s, 1)
                y = y + jnp.where((lane & s) != 0, fwd, bwd)
                s *= 2
            parts.append((pqj / (y + 1e-6)).astype(jnp.bfloat16))
        pqn = jnp.concatenate(parts, axis=1)
        up = jnp.dot(xt, w3_v[:, pl.ds(0, fc)], preferred_element_type=jnp.float32)
        a = jnp.dot(pqn, m_v[...], preferred_element_type=jnp.float32)
        h = (gate * jax.nn.sigmoid(gate) * up).astype(jnp.bfloat16)
        b = jnp.dot(h, w2_v[pl.ds(0, fc), :], preferred_element_type=jnp.float32)
        for c in range(1, F // fc):
            c0 = c * fc
            gate = jnp.dot(xt, w1_v[:, pl.ds(c0, fc)], preferred_element_type=jnp.float32)
            up = jnp.dot(xt, w3_v[:, pl.ds(c0, fc)], preferred_element_type=jnp.float32)
            h = (gate * jax.nn.sigmoid(gate) * up).astype(jnp.bfloat16)
            b = b + jnp.dot(h, w2_v[pl.ds(c0, fc), :], preferred_element_type=jnp.float32)
        gw = gw_v[...]
        g = jax.nn.sigmoid(jnp.sum(xt.astype(jnp.float32) * gw, axis=-1, keepdims=True))
        o_ref[...] = (g * a + (1.0 - g) * b).astype(o_ref.dtype)


@jax.jit
def pallas_gated_mix__linear_attn_block__glu_gated_swiglu__prompt_kernel(
    A_x: jax.Array,
    A_wqkv: jax.Array,
    A_wo: jax.Array,
    B_x: jax.Array,
    B_w1: jax.Array,
    B_w3: jax.Array,
    B_w2: jax.Array,
    gate_w: jax.Array,
):
    B, S, D = A_x.shape
    F = B_w1.shape[1]
    t1 = 512
    kc = 512
    tm = 256
    fc = 896
    nt1 = S // t1
    nc1 = D // kc
    n1 = nt1 * nc1
    n2 = S // tm
    x2 = A_x.reshape(S, D)
    gw2 = gate_w
    bf = jnp.bfloat16

    kernel = functools.partial(_kernel, t1=t1, nt1=nt1, kc=kc, nc1=nc1, tm=tm, n2=n2,
                               S=S, D=D, F=F, fc=fc)
    any_spec = pl.BlockSpec(memory_space=pl.ANY)
    out = pl.pallas_call(
        kernel,
        grid=(n1 + n2,),
        in_specs=[any_spec] * 6 + [pl.BlockSpec((D,), lambda i: (0,))],
        out_specs=pl.BlockSpec((tm, D), lambda i: (jnp.maximum(i - n1, 0), 0)),
        out_shape=jax.ShapeDtypeStruct((S, D), A_x.dtype),
        scratch_shapes=[
            pltpu.VMEM((S, D), bf),
            pltpu.VMEM((D, D), bf),
            pltpu.VMEM((nc1, D, kc), bf),
            pltpu.VMEM((D, D), bf),
            pltpu.VMEM((D, D), bf),
            pltpu.VMEM((D, F), bf),
            pltpu.VMEM((D, F), bf),
            pltpu.VMEM((F, D), bf),
            pltpu.VMEM((nc1, kc, D), jnp.float32),
            pltpu.VMEM((nc1, 1, kc), jnp.float32),
            pltpu.VMEM((D, D), bf),
            pltpu.VMEM((1, D), jnp.float32),
            pltpu.SemaphoreType.DMA((nt1 + nc1 + 6,)),
        ],
        compiler_params=pltpu.CompilerParams(
            dimension_semantics=("arbitrary",),
            vmem_limit_bytes=100 * 1024 * 1024,
        ),
    )(x2, A_wqkv, A_wo, B_w1, B_w3, B_w2, gw2)
    return out.reshape(B, S, D)
```

```python
import functools

import jax
import jax.numpy as jnp
from jax import lax
import jax.experimental.pallas as pl
import jax.experimental.pallas.tpu as pltpu

HEAD_DIM = 32
LANE = 128


def _phi(t):
    return jnp.where(t > 0, t + 1.0, jnp.exp(t)) + 1e-6


def _kernel(x_hbm, wqkv_hbm, wo_hbm, w1_hbm, w3_hbm, w2_hbm, gw_ref,
            o_ref,
            x_v, wq_v, wk_v, wv_v, wo_v, w1_v, w3_v, w2_v,
            p_acc, z_acc, m_v, gw_v, sems,
            *, t1, nt1, kc, nc1, tm, S, D, F, fc):
    i = pl.program_id(0)
    n1 = nt1 * nc1
    nblk = D // LANE
    bpc = kc // LANE

    def x_copy(t):
        return pltpu.make_async_copy(
            x_hbm.at[pl.ds(t * t1, t1), :], x_v.at[pl.ds(t * t1, t1), :], sems.at[t])

    def wk_copy(c):
        return pltpu.make_async_copy(
            wqkv_hbm.at[:, pl.ds(D + c * kc, kc)], wk_v.at[c], sems.at[nt1 + c])

    sb = nt1 + nc1

    def late_copies():
        cps = [
            pltpu.make_async_copy(wqkv_hbm.at[:, pl.ds(2 * D + j * LANE, LANE)],
                                  wv_v.at[j], sems.at[sb + j])
            for j in range(nblk)
        ]
        s2 = sb + nblk
        return cps + [
            pltpu.make_async_copy(wo_hbm, wo_v, sems.at[s2]),
            pltpu.make_async_copy(wqkv_hbm.at[:, pl.ds(0, D)], wq_v, sems.at[s2 + 1]),
            pltpu.make_async_copy(w1_hbm, w1_v, sems.at[s2 + 2]),
            pltpu.make_async_copy(w3_hbm, w3_v, sems.at[s2 + 3]),
            pltpu.make_async_copy(w2_hbm, w2_v, sems.at[s2 + 4]),
        ]

    @pl.when(i == 0)
    def _():
        x_copy(0).start()
        wk_copy(0).start()
        for t in range(1, nt1):
            x_copy(t).start()
        for c in range(1, nc1):
            wk_copy(c).start()
        for c in late_copies():
            c.start()

        def zero(j, carry):
            p_acc[j] = jnp.zeros((LANE, D), jnp.float32)
            return carry

        lax.fori_loop(0, nblk, zero, 0)
        z_acc[...] = jnp.zeros_like(z_acc)
        gw_v[...] = gw_ref[...].astype(jnp.float32).reshape(1, D)

    @pl.when(i < n1)
    def _():
        c = i // nt1
        t = i % nt1
        for tt in range(nt1):
            @pl.when(i == tt)
            def _():
                x_copy(tt).wait()
        for cc in range(nc1):
            @pl.when(i == cc * nt1)
            def _():
                wk_copy(cc).wait()
        r0 = pl.multiple_of(t * t1, t1)
        xt = x_v[pl.ds(r0, t1), :]
        k = jnp.dot(xt, wk_v[c], preferred_element_type=jnp.float32)
        pk = _phi(k).astype(jnp.bfloat16)
        z_acc[c] += jnp.sum(pk.astype(jnp.float32), axis=0, keepdims=True)
        p = lax.dot_general(
            pk, xt, (((0,), (0,)), ((), ())), preferred_element_type=jnp.float32)
        b0 = pl.multiple_of(c * bpc, bpc)
        p_acc[pl.ds(b0, bpc)] += p.reshape(bpc, LANE, D)

    @pl.when(i == n1)
    def _():
        for c in late_copies():
            c.wait()
        rr = lax.broadcasted_iota(jnp.int32, (LANE, LANE), 0) // HEAD_DIM
        cc = lax.broadcasted_iota(jnp.int32, (LANE, LANE), 1) // HEAD_DIM
        diag = rr == cc

        def fold(j, carry):
            j0 = pl.multiple_of(j * LANE, LANE)
            kvj = jnp.dot(p_acc[j].astype(jnp.bfloat16), wv_v[j],
                          preferred_element_type=jnp.float32)
            kvj = jnp.where(diag, kvj, 0.0).astype(jnp.bfloat16)
            m_v[pl.ds(j0, LANE), :] = jnp.dot(
                kvj, wo_v[pl.ds(j0, LANE), :],
                preferred_element_type=jnp.float32).astype(jnp.bfloat16)
            return carry

        lax.fori_loop(0, nblk, fold, 0, unroll=2)

    @pl.when(i >= n1)
    def _():
        r0 = pl.multiple_of((i - n1) * tm, tm)
        xt = x_v[pl.ds(r0, tm), :]
        q = jnp.dot(xt, wq_v[...], preferred_element_type=jnp.float32)
        gate = jnp.dot(xt, w1_v[:, pl.ds(0, fc)], preferred_element_type=jnp.float32)
        pq = _phi(q).astype(jnp.bfloat16)
        parts = []
        lane = lax.broadcasted_iota(jnp.int32, (tm, LANE), 1)
        for j in range(nblk):
            pqj = pq[:, j * LANE:(j + 1) * LANE].astype(jnp.float32)
            y = pqj * z_acc[j // bpc, :, pl.ds((j % bpc) * LANE, LANE)]
            s = 1
            while s < HEAD_DIM:
                fwd = pltpu.roll(y, s, 1)
                bwd = pltpu.roll(y, LANE - s, 1)
                y = y + jnp.where((lane & s) != 0, fwd, bwd)
                s *= 2
            parts.append((pqj / (y + 1e-6)).astype(jnp.bfloat16))
        pqn = jnp.concatenate(parts, axis=1)
        up = jnp.dot(xt, w3_v[:, pl.ds(0, fc)], preferred_element_type=jnp.float32)
        a = jnp.dot(pqn, m_v[...], preferred_element_type=jnp.float32)
        h = (gate * jax.nn.sigmoid(gate) * up).astype(jnp.bfloat16)
        b = jnp.dot(h, w2_v[pl.ds(0, fc), :], preferred_element_type=jnp.float32)
        for c in range(1, F // fc):
            c0 = c * fc
            gate = jnp.dot(xt, w1_v[:, pl.ds(c0, fc)], preferred_element_type=jnp.float32)
            up = jnp.dot(xt, w3_v[:, pl.ds(c0, fc)], preferred_element_type=jnp.float32)
            h = (gate * jax.nn.sigmoid(gate) * up).astype(jnp.bfloat16)
            b = b + jnp.dot(h, w2_v[pl.ds(c0, fc), :], preferred_element_type=jnp.float32)
        gw = gw_v[...]
        g = jax.nn.sigmoid(jnp.sum(xt.astype(jnp.float32) * gw, axis=-1, keepdims=True))
        o_ref[...] = (g * a + (1.0 - g) * b).astype(o_ref.dtype)


@jax.jit
def pallas_gated_mix__linear_attn_block__glu_gated_swiglu__prompt_kernel(
    A_x: jax.Array,
    A_wqkv: jax.Array,
    A_wo: jax.Array,
    B_x: jax.Array,
    B_w1: jax.Array,
    B_w3: jax.Array,
    B_w2: jax.Array,
    gate_w: jax.Array,
):
    B, S, D = A_x.shape
    F = B_w1.shape[1]
    t1 = 512
    kc = 512
    tm = 256
    fc = 896
    nt1 = S // t1
    nc1 = D // kc
    n1 = nt1 * nc1
    n2 = S // tm
    nblk = D // LANE
    x2 = A_x.reshape(S, D)
    bf = jnp.bfloat16

    kernel = functools.partial(_kernel, t1=t1, nt1=nt1, kc=kc, nc1=nc1, tm=tm,
                               S=S, D=D, F=F, fc=fc)
    any_spec = pl.BlockSpec(memory_space=pl.ANY)
    out = pl.pallas_call(
        kernel,
        grid=(n1 + n2,),
        in_specs=[any_spec] * 6 + [pl.BlockSpec((D,), lambda i: (0,))],
        out_specs=pl.BlockSpec((tm, D), lambda i: (jnp.maximum(i - n1, 0), 0)),
        out_shape=jax.ShapeDtypeStruct((S, D), A_x.dtype),
        scratch_shapes=[
            pltpu.VMEM((S, D), bf),
            pltpu.VMEM((D, D), bf),
            pltpu.VMEM((nc1, D, kc), bf),
            pltpu.VMEM((nblk, D, LANE), bf),
            pltpu.VMEM((D, D), bf),
            pltpu.VMEM((D, F), bf),
            pltpu.VMEM((D, F), bf),
            pltpu.VMEM((F, D), bf),
            pltpu.VMEM((nblk, LANE, D), jnp.float32),
            pltpu.VMEM((nc1, 1, kc), jnp.float32),
            pltpu.VMEM((D, D), bf),
            pltpu.VMEM((1, D), jnp.float32),
            pltpu.SemaphoreType.DMA((nt1 + nc1 + nblk + 5,)),
        ],
        compiler_params=pltpu.CompilerParams(
            dimension_semantics=("arbitrary",),
            vmem_limit_bytes=100 * 1024 * 1024,
        ),
    )(x2, A_wqkv, A_wo, B_w1, B_w3, B_w2, gate_w)
    return out.reshape(B, S, D)
```

```python
import functools

import jax
import jax.numpy as jnp
from jax import lax
import jax.experimental.pallas as pl
import jax.experimental.pallas.tpu as pltpu

HEAD_DIM = 32
LANE = 128


def _phi(t):
    return jnp.where(t > 0, t + 1.0, jnp.exp(t)) + 1e-6


def _kernel(x_hbm, wqkv_hbm, wo_hbm, w1_hbm, w3_hbm, w2_hbm, gw_ref,
            o_hbm,
            x_v, wq_v, wk_v, wv_v, wo_v, w1_v, w3_v, w2_v,
            p_acc, z_acc, m_v, o_buf, sems, osems,
            *, t1, nt1, kc, nc1, tm, n2, S, D, F, fc):
    n1 = nt1 * nc1
    nblk = D // LANE
    bpc = kc // LANE

    def x_copy(t):
        return pltpu.make_async_copy(
            x_hbm.at[pl.ds(t * t1, t1), :], x_v.at[pl.ds(t * t1, t1), :], sems.at[t])

    def wk_copy(c):
        return pltpu.make_async_copy(
            wqkv_hbm.at[:, pl.ds(D + c * kc, kc)], wk_v.at[c], sems.at[nt1 + c])

    sb = nt1 + nc1

    def late_copies():
        cps = [
            pltpu.make_async_copy(wqkv_hbm.at[:, pl.ds(2 * D + j * LANE, LANE)],
                                  wv_v.at[j], sems.at[sb + j])
            for j in range(nblk)
        ]
        s2 = sb + nblk
        return cps + [
            pltpu.make_async_copy(wo_hbm, wo_v, sems.at[s2]),
            pltpu.make_async_copy(wqkv_hbm.at[:, pl.ds(0, D)], wq_v, sems.at[s2 + 1]),
            pltpu.make_async_copy(w1_hbm, w1_v, sems.at[s2 + 2]),
            pltpu.make_async_copy(w3_hbm, w3_v, sems.at[s2 + 3]),
            pltpu.make_async_copy(w2_hbm, w2_v, sems.at[s2 + 4]),
        ]

    def out_copy(i, slot):
        r0 = pl.multiple_of(i * tm, tm)
        return pltpu.make_async_copy(
            o_buf.at[slot], o_hbm.at[pl.ds(r0, tm), :], osems.at[slot])

    x_copy(0).start()
    wk_copy(0).start()
    for t in range(1, nt1):
        x_copy(t).start()
    for c in range(1, nc1):
        wk_copy(c).start()
    for c in late_copies():
        c.start()

    def zero(j, carry):
        p_acc[j] = jnp.zeros((LANE, D), jnp.float32)
        return carry

    lax.fori_loop(0, nblk, zero, 0)
    z_acc[...] = jnp.zeros_like(z_acc)

    def phase1(i, carry):
        c = i // nt1
        t = i % nt1
        for tt in range(nt1):
            @pl.when(i == tt)
            def _():
                x_copy(tt).wait()
        for cc in range(nc1):
            @pl.when(i == cc * nt1)
            def _():
                wk_copy(cc).wait()
        r0 = pl.multiple_of(t * t1, t1)
        xt = x_v[pl.ds(r0, t1), :]
        k = jnp.dot(xt, wk_v[c], preferred_element_type=jnp.float32)
        pk = _phi(k).astype(jnp.bfloat16)
        z_acc[c] += jnp.sum(pk.astype(jnp.float32), axis=0, keepdims=True)
        p = lax.dot_general(
            pk, xt, (((0,), (0,)), ((), ())), preferred_element_type=jnp.float32)
        b0 = pl.multiple_of(c * bpc, bpc)
        p_acc[pl.ds(b0, bpc)] += p.reshape(bpc, LANE, D)
        return carry

    lax.fori_loop(0, n1, phase1, 0)

    for c in late_copies():
        c.wait()
    rr = lax.broadcasted_iota(jnp.int32, (LANE, LANE), 0) // HEAD_DIM
    cc = lax.broadcasted_iota(jnp.int32, (LANE, LANE), 1) // HEAD_DIM
    diag = rr == cc

    def fold(j, carry):
        j0 = pl.multiple_of(j * LANE, LANE)
        kvj = jnp.dot(p_acc[j].astype(jnp.bfloat16), wv_v[j],
                      preferred_element_type=jnp.float32)
        kvj = jnp.where(diag, kvj, 0.0).astype(jnp.bfloat16)
        m_v[pl.ds(j0, LANE), :] = jnp.dot(
            kvj, wo_v[pl.ds(j0, LANE), :],
            preferred_element_type=jnp.float32).astype(jnp.bfloat16)
        return carry

    lax.fori_loop(0, nblk, fold, 0, unroll=2)

    def phase2(i, carry):
        slot = i % 2

        @pl.when(i >= 2)
        def _():
            out_copy(i - 2, slot).wait()

        r0 = pl.multiple_of(i * tm, tm)
        xt = x_v[pl.ds(r0, tm), :]
        q = jnp.dot(xt, wq_v[...], preferred_element_type=jnp.float32)
        gate = jnp.dot(xt, w1_v[:, pl.ds(0, fc)], preferred_element_type=jnp.float32)
        pq = _phi(q).astype(jnp.bfloat16)
        parts = []
        lane = lax.broadcasted_iota(jnp.int32, (tm, LANE), 1)
        for j in range(nblk):
            pqj = pq[:, j * LANE:(j + 1) * LANE].astype(jnp.float32)
            y = pqj * z_acc[j // bpc, :, pl.ds((j % bpc) * LANE, LANE)]
            s = 1
            while s < HEAD_DIM:
                fwd = pltpu.roll(y, s, 1)
                bwd = pltpu.roll(y, LANE - s, 1)
                y = y + jnp.where((lane & s) != 0, fwd, bwd)
                s *= 2
            parts.append((pqj / (y + 1e-6)).astype(jnp.bfloat16))
        pqn = jnp.concatenate(parts, axis=1)
        up = jnp.dot(xt, w3_v[:, pl.ds(0, fc)], preferred_element_type=jnp.float32)
        a = jnp.dot(pqn, m_v[...], preferred_element_type=jnp.float32)
        h = (gate * jax.nn.sigmoid(gate) * up).astype(jnp.bfloat16)
        b = jnp.dot(h, w2_v[pl.ds(0, fc), :], preferred_element_type=jnp.float32)
        for c in range(1, F // fc):
            c0 = c * fc
            gate = jnp.dot(xt, w1_v[:, pl.ds(c0, fc)], preferred_element_type=jnp.float32)
            up = jnp.dot(xt, w3_v[:, pl.ds(c0, fc)], preferred_element_type=jnp.float32)
            h = (gate * jax.nn.sigmoid(gate) * up).astype(jnp.bfloat16)
            b = b + jnp.dot(h, w2_v[pl.ds(c0, fc), :], preferred_element_type=jnp.float32)
        gw = gw_ref[...].astype(jnp.float32)
        g = jax.nn.sigmoid(jnp.sum(xt.astype(jnp.float32) * gw, axis=-1, keepdims=True))
        o_buf[slot] = (g * a + (1.0 - g) * b).astype(o_buf.dtype)
        out_copy(i, slot).start()
        return carry

    lax.fori_loop(0, n2, phase2, 0)
    out_copy(n2 - 2, (n2 - 2) % 2).wait()
    out_copy(n2 - 1, (n2 - 1) % 2).wait()


@jax.jit
def pallas_gated_mix__linear_attn_block__glu_gated_swiglu__prompt_kernel(
    A_x: jax.Array,
    A_wqkv: jax.Array,
    A_wo: jax.Array,
    B_x: jax.Array,
    B_w1: jax.Array,
    B_w3: jax.Array,
    B_w2: jax.Array,
    gate_w: jax.Array,
):
    B, S, D = A_x.shape
    F = B_w1.shape[1]
    t1 = 512
    kc = 512
    tm = 256
    fc = 896
    nt1 = S // t1
    nc1 = D // kc
    n2 = S // tm
    nblk = D // LANE
    x2 = A_x.reshape(S, D)
    bf = jnp.bfloat16

    kernel = functools.partial(_kernel, t1=t1, nt1=nt1, kc=kc, nc1=nc1, tm=tm, n2=n2,
                               S=S, D=D, F=F, fc=fc)
    any_spec = pl.BlockSpec(memory_space=pl.ANY)
    out = pl.pallas_call(
        kernel,
        in_specs=[any_spec] * 6 + [pl.BlockSpec(memory_space=pltpu.VMEM)],
        out_specs=any_spec,
        out_shape=jax.ShapeDtypeStruct((S, D), A_x.dtype),
        scratch_shapes=[
            pltpu.VMEM((S, D), bf),
            pltpu.VMEM((D, D), bf),
            pltpu.VMEM((nc1, D, kc), bf),
            pltpu.VMEM((nblk, D, LANE), bf),
            pltpu.VMEM((D, D), bf),
            pltpu.VMEM((D, F), bf),
            pltpu.VMEM((D, F), bf),
            pltpu.VMEM((F, D), bf),
            pltpu.VMEM((nblk, LANE, D), jnp.float32),
            pltpu.VMEM((nc1, 1, kc), jnp.float32),
            pltpu.VMEM((D, D), bf),
            pltpu.VMEM((2, tm, D), A_x.dtype),
            pltpu.SemaphoreType.DMA((nt1 + nc1 + nblk + 5,)),
            pltpu.SemaphoreType.DMA((2,)),
        ],
        compiler_params=pltpu.CompilerParams(
            vmem_limit_bytes=100 * 1024 * 1024,
        ),
    )(x2, A_wqkv, A_wo, B_w1, B_w3, B_w2, gate_w.reshape(1, D))
    return out.reshape(B, S, D)
```
